```python
import os as _os
_os.environ.setdefault("JAX_PLATFORMS", "cpu")
import jax
import jax.numpy as jnp

def _softmax(x, axis=-1):
    return jax.nn.softmax(x, axis=axis)
def _gelu(x):
    return jax.nn.gelu(x, approximate=True)
def _silu(x):
    return jax.nn.silu(x)
def _sigmoid(x):
    return jax.nn.sigmoid(x)
def _layernorm(x, axis=-1, eps=1e-5):
    m = jnp.mean(x, axis=axis, keepdims=True)
    v = jnp.var(x, axis=axis, keepdims=True)
    return (x - m) / jnp.sqrt(v + eps)
def _scatter_add(tgt, idx, src, axis=0):
    return tgt.at[idx].add(src)
def _segment_sum(src, seg, n):
    return jax.ops.segment_sum(src, seg, n)
class _Rng:
    def __init__(self, key):
        self._k = key
    def _next(self):
        self._k, sub = jax.random.split(self._k)
        return sub
    def normal(self, shape):
        return jax.random.normal(self._next(), shape, dtype=jnp.bfloat16)
    def randint(self, lo, hi, shape):
        return jax.random.randint(self._next(), shape, lo, hi, dtype=jnp.int32)
    def uniform(self, shape, lo=0.0, hi=1.0):
        return jax.random.uniform(self._next(), shape, jnp.bfloat16, lo, hi)
    def permutation(self, n):
        return jax.random.permutation(self._next(), n)


kernel_name = 'sequential_preLN__mha_block__moe_arch_mod__prompt'

def setup_inputs():
    _rng = _Rng(jax.random.key(int.from_bytes(__import__("os").urandom(4), "little")))
    _w = (lambda a: (lambda t: t.astype(jnp.bfloat16) if jnp.issubdtype(t.dtype, jnp.floating) else t)(jnp.asarray(a)))
    def _A_setup():
        B, S, D, H = 1, 2048, 512, 32
        return {
            "x": _w((lambda *s: _rng.normal(s) * 0.05)(B, S, D)),
            "wqkv": _w((lambda *s: _rng.normal(s) * 0.05)(D, 3 * D)),
            "wo": _w((lambda *s: _rng.normal(s) * 0.05)(D, D)),
        }
    _A_in = _A_setup()

    def _B_setup():
        B, S, D, F, C = 1, 2048, 512, 1792, 2
        return {
            "x": _w((lambda *s: _rng.normal(s) * 0.05)(B, S, D)),
            "w_r": _w((lambda *s: _rng.normal(s) * 0.05)(D)),
            "w_gate": _w((lambda *s: _rng.normal(s) * 0.05)(D, F)),
            "w_up": _w((lambda *s: _rng.normal(s) * 0.05)(D, F)),
            "w_down": _w((lambda *s: _rng.normal(s) * 0.05)(F, D)),
        }
    _B_in = _B_setup()

    return {
        "A_x": _A_in["x"],
        "A_wqkv": _A_in["wqkv"],
        "A_wo": _A_in["wo"],
        "B_x": _B_in["x"],
        "B_w_r": _B_in["w_r"],
        "B_w_gate": _B_in["w_gate"],
        "B_w_up": _B_in["w_up"],
        "B_w_down": _B_in["w_down"],
    }

def reference(A_x, A_wqkv, A_wo, B_x, B_w_r, B_w_gate, B_w_up, B_w_down):
    def _A_ref(x, wqkv, wo):
        B, S, D = x.shape
        H = 32
        Dh = D // H
        qkv = (lambda x, *d: x.transpose(*d))((x @ wqkv).reshape(B, S, 3, H, Dh), 2, 0, 3, 1, 4)
        q, k, v = qkv[0], qkv[1], qkv[2]
        scores = jnp.einsum("bhqd,bhkd->bhqk", q, k) * (Dh ** -0.5)
        p = _softmax(scores, axis=-1)
        o = jnp.einsum("bhqk,bhkd->bhqd", p, v)
        return (lambda x, *d: x.transpose(*d))(o, 0, 2, 1, 3).reshape(B, S, D) @ wo

    def _B_ref(x, w_r, w_gate, w_up, w_down):
        B, S, D = x.shape
        C = 2
        r = x @ w_r
        idx = jnp.argsort(-r, axis=-1)[:, :C]
        idx_e = jnp.repeat(idx.reshape(B, C, 1), D, axis=2)
        x_sel = jnp.take_along_axis(x, idx_e, axis=1)
        g = _silu(x_sel @ w_gate)
        u = x_sel @ w_up
        y = (g * u) @ w_down
        r_sel = _sigmoid(jnp.take_along_axis(r, idx, axis=1))
        y = y * r_sel.reshape(B, C, 1)
        b_off = (jnp.arange(B) * S).reshape(B, 1)
        flat_idx = (idx + b_off).reshape(B * C)
        zero = (x * 0.0).reshape(B * S, D)
        upd = _scatter_add(zero, flat_idx, y.reshape(B * C, D), axis=0)
        return x + upd.reshape(B, S, D)

    x = A_x
    h = x + _A_ref(_layernorm(x, axis=-1), A_wqkv, A_wo)
    h2 = h + _B_ref(_layernorm(h, axis=-1), B_w_r, B_w_gate, B_w_up, B_w_down)
    return h2
```

```python
import functools

import jax
import jax.numpy as jnp
from jax import lax
import jax.experimental.pallas as pl
import jax.experimental.pallas.tpu as pltpu

S = 2048
D = 512
H = 32
DH = 16
F = 1792
W = 512
CH = 128
NC = S // CH
NQ = S // W
TC = 512
EPS = 1e-5
QSCALE = DH ** -0.5 * 1.4426950408889634
L_MIN = 2.0 ** -50

BF = jnp.bfloat16
F32 = jnp.float32
U32 = jnp.uint32
I32 = jnp.int32


def _pk(x):
    return pltpu.bitcast(x, U32)


def _upk(x):
    return pltpu.bitcast(x, BF)


def _dot(a, b, ca=1, cb=0):
    return lax.dot_general(a, b, (((ca,), (cb,)), ((), ())), preferred_element_type=F32)


def _layernorm(x):
    mu = jnp.sum(x, axis=-1, keepdims=True) * (1.0 / D)
    xc = x - mu
    var = jnp.sum(xc * xc, axis=-1, keepdims=True) * (1.0 / D)
    return xc * lax.rsqrt(var + EPS)


def make_kernel(VP=(4, 12), PIN=0):
    G = len(VP)
    vpu_blocks = [15 - p for p in VP]
    mxu_blocks = [b for b in range(15, -1, -1) if b not in vpu_blocks]
    KM = 8 * len(mxu_blocks)
    assert KM % 16 == 0

    def kernel(x_hbm, wqkv_hbm, wo_hbm, wr_hbm, wg_hbm, wu_hbm, wd_hbm, out_hbm,
               x_v, wqkv_v, wo_v, wr_v, wg_v, wu_v, wd_v, out_v,
               wt_s, qt_s, vt_s, xn_s, kv_s, kf_s, kap_s, ot_s,
               ka_s, kb_s, qa_s, nu_s, qb_s, a_s, hn_s, zero_s, zi_s, sem, osem):
        def x_cp(i):
            return pltpu.make_async_copy(x_hbm.at[pl.ds(i * TC, TC)], x_v.at[pl.ds(i * TC, TC)], sem.at[i])

        def w_cp(i):
            return pltpu.make_async_copy(wqkv_hbm.at[:, pl.ds(i * D, D)], wqkv_v.at[i], sem.at[4 + i])

        late = [pltpu.make_async_copy(s_, d_, sem.at[7 + i]) for i, (s_, d_) in enumerate(
            [(wo_hbm, wo_v), (wr_hbm, wr_v), (wg_hbm, wg_v), (wu_hbm, wu_v), (wd_hbm, wd_v)])]

        x_cp(0).start()
        w_cp(1).start()
        w_cp(0).start()
        w_cp(2).start()
        for i in range(1, S // TC):
            x_cp(i).start()
        for c in late:
            c.start()

        zero_s[...] = jnp.zeros_like(zero_s)
        for i in range(2 * NQ * NC):
            zi_s[i] = pl.program_id(0)

        kmax = jnp.zeros((8, D), F32)
        for i in range(S // TC):
            x_cp(i).wait()
            xn = _layernorm(x_v[pl.ds(i * TC, TC), :].astype(F32)).astype(BF)
            xn_s[i * TC // 2:(i + 1) * TC // 2, :] = _pk(xn)
            if i == 0:
                w_cp(1).wait()
            k = _dot(xn, wqkv_v[1])
            kmax = jnp.maximum(kmax, jnp.max(jnp.abs(k).reshape(TC // 8, 8, D), axis=0))
            kfp = _pk(k.astype(BF))
            for cc in range(TC // CH):
                c = i * (TC // CH) + cc
                blk = lambda b: k[cc * CH + 8 * b:cc * CH + 8 * b + 8]
                km = _pk(jnp.concatenate([blk(b) for b in mxu_blocks], axis=0).astype(BF))
                lane_k = lax.broadcasted_iota(I32, (KM // 2, 128), 1)
                for g in range(D // 128):
                    kg = km[:, g * 128:(g + 1) * 128]
                    for j in range(8):
                        kr = kg if j == 0 else pltpu.roll(kg, 128 - DH * j, 1)
                        ka_s[8 * g + j, c * KM // 2:(c + 1) * KM // 2, :] = jnp.where(lane_k == DH, U32(0x3F803F80), kr)
                    for j, b in enumerate(vpu_blocks):
                        r = 8 * (c * G + j)
                        kv_s[g, r:r + 8, :] = blk(b)[:, g * 128:(g + 1) * 128]
            for g in range(D // 128):
                kf_s[g, i * TC // 2:(i + 1) * TC // 2, :] = kfp[:, g * 128:(g + 1) * 128]
        kmax = jnp.max(kmax, axis=0, keepdims=True)
        for g in range(D // 128):
            kap_s[g * 128:(g + 1) * 128, :] = jnp.broadcast_to(kmax[:, g * 128:(g + 1) * 128], (128, 128)).T
        w_cp(0).wait()
        wt_s[0:D // 2, :] = _pk(wqkv_v[0].T)
        w_cp(2).wait()
        wt_s[D // 2:D, :] = _pk(wqkv_v[2].T)
        sub16 = lax.broadcasted_iota(I32, (DH, TC), 0)
        for i in range(S // TC):
            cols = slice(i * TC, (i + 1) * TC)
            qv = _dot(_upk(wt_s[...]), _upk(xn_s[i * TC // 2:(i + 1) * TC // 2, :]), 1, 1)
            vt_s[:, cols] = _pk(qv[D:].astype(BF))
            for h in range(H):
                q = qv[h * DH:(h + 1) * DH] * QSCALE
                qt_s[h * DH:(h + 1) * DH, cols] = q
                kap = kap_s[h * DH:(h + 1) * DH, :]
                nu = -jnp.sum(jnp.abs(q) * jnp.concatenate([kap] * (TC // 128), axis=1), axis=0, keepdims=True)
                nu = nu.astype(BF).astype(F32)
                nu_s[h, :, cols] = jnp.broadcast_to(nu, (8, TC))
                qa = jnp.concatenate([q, jnp.where(sub16 == 0, nu, 0.0)], axis=0)
                qa_s[h, :, cols] = _pk(qa.astype(BF))

        NP = NC * G // NQ * 8

        def rolled_keys(h, u):
            return pltpu.roll(kv_s[h // 8, u * NP:(u + 1) * NP, :], (128 - DH * (h % 8)) % 128, 1)

        if G:
            for u in range(NQ):
                kv = rolled_keys(0, u)
                for d in range(DH):
                    kb_s[0][0, d, u * NP:(u + 1) * NP, :] = jnp.broadcast_to(kv[:, d:d + 1], (NP, 128))

        def heads(hh, bad):
            acc = {}

            def front(e, u, c):
                h = hh * 2 + e
                z = zi_s[(e * NQ + u) * NC + c]
                cols = slice(u * W, (u + 1) * W)
                kc = _upk(ka_s[h, c * KM // 2:(c + 1) * KM // 2, 0:2 * DH])
                s = _dot(kc, _upk(qa_s[h, :, cols]))
                blocks = {b: s[8 * j:8 * j + 8] for j, b in enumerate(mxu_blocks)}
                if G:
                    if c == 0:
                        acc["kv"] = rolled_keys(jnp.minimum(h + 1, H - 1), u)
                    kb_s[1 - e][0, c, u * NP:(u + 1) * NP, :] = jnp.broadcast_to(acc["kv"][:, c:c + 1], (NP, 128))
                    if PIN:
                        acc["pin", e, u, c] = kb_s[1 - e][z, c, u * NP:u * NP + 8, :]
                    a = [nu_s[h + z, :, cols]] * G
                    fresh_q = c == 0
                    if fresh_q:
                        q = qt_s[pl.ds(pl.multiple_of(h * DH, DH), DH), cols]
                    for d in range(DH):
                        if fresh_q:
                            qd = jnp.broadcast_to(q[d:d + 1], (8, W))
                            qb_s[u][0, d] = qd
                        else:
                            qd = qb_s[u][z, d]
                        for j in range(G):
                            r = 8 * (c * G + j)
                            kd = kb_s[e][z, d, r:r + 8, :]
                            a[j] = a[j] + jnp.concatenate([kd] * (W // 128), axis=1) * qd
                    blocks.update(zip(vpu_blocks, a))
                p = {b: jnp.exp2(blocks[b]) for b in range(15, -1, -1)}
                l = acc.get(("l", e, u))
                for b in range(15, -1, -1):
                    l = p[b] if l is None else l + p[b]
                acc["l", e, u] = l
                return jnp.concatenate([p[b] for b in range(16)], axis=0)

            def back(e, u, c, p, bad):
                r8 = pl.multiple_of((hh * 2 + e) * 8, 8)
                if c == 0:
                    acc["o"] = zero_s[...]
                vc = vt_s[pl.ds(r8, 8), c * CH:(c + 1) * CH]
                if G and PIN:
                    vc = vc | (pltpu.bitcast(acc["pin", e, u, c], U32) & pltpu.bitcast(zero_s[0:8, 0:128], U32))
                acc["o"] = acc["o"] + _dot(_upk(vc), p)
                if c == NC - 1:
                    l = jnp.sum(acc["l", e, u], axis=0, keepdims=True)
                    bad = jnp.where(l >= L_MIN, bad, 1.0)
                    ot_s[pl.ds(r8, 8), u * W:(u + 1) * W] = _pk((acc["o"] * (1.0 / l)).astype(BF))
                return bad

            pend = None
            for e in range(2):
                for u in range(NQ):
                    for c in range(NC):
                        p = front(e, u, c)
                        if pend is not None:
                            bad = back(*pend, bad)
                        pend = (e, u, c, p)
            return back(*pend, bad)

        bad = lax.fori_loop(0, H // 2, heads, jnp.zeros((1, W), F32))

        @pl.when(jnp.max(bad) > 0.0)
        def _exact():
            def body(t, carry):
                h = t // (S // 128)
                q0 = pl.multiple_of((t % (S // 128)) * 128, 128)
                g = h // 8
                qg = qt_s[pl.ds(pl.multiple_of(g * 128, 128), 128), pl.ds(q0, 128)]
                rows = lax.broadcasted_iota(I32, (128, 128), 0) // DH
                qg = jnp.where(rows == h % 8, qg, 0.0).astype(BF)
                kg = _upk(kf_s[g])
                lanes = lax.broadcasted_iota(I32, kg.shape, 1) // DH
                kg = jnp.where(lanes == h % 8, kg, jnp.zeros_like(kg))
                s = _dot(kg, qg)
                p = jnp.exp2(s - jnp.max(s, axis=0, keepdims=True))
                l = jnp.sum(p, axis=0, keepdims=True)
                r8 = pl.multiple_of(h * 8, 8)
                o = _dot(_upk(vt_s[pl.ds(r8, 8), :]), p.astype(BF))
                ot_s[pl.ds(r8, 8), pl.ds(q0, 128)] = _pk((o * (1.0 / l)).astype(BF))
                return carry
            lax.fori_loop(0, H * (S // 128), body, 0)

        for c in late:
            c.wait()
        wr = wr_v[...].astype(F32)
        neg = jnp.full((8, 1), -jnp.inf, F32)
        m1 = m2 = neg
        i1 = i2 = jnp.zeros((8, 1), I32)
        row8 = lax.broadcasted_iota(I32, (8, 1), 0)

        def o_cp(i):
            return pltpu.make_async_copy(out_v.at[pl.ds(i * TC, TC)], out_hbm.at[pl.ds(i * TC, TC)], osem.at[i])

        for i in range(S // TC):
            att = _dot(_upk(ot_s[:, i * TC:(i + 1) * TC]), wo_v[...], 0, 0)
            h1 = (x_v[pl.ds(i * TC, TC), :].astype(F32) + att).astype(BF).astype(F32)
            hn = _layernorm(h1).astype(BF).astype(F32)
            a_s[i * TC:(i + 1) * TC, :] = h1
            hn_s[i * TC:(i + 1) * TC, :] = hn
            out_v[pl.ds(i * TC, TC), :] = (h1 + hn).astype(BF)
            o_cp(i).start()
            r = jnp.sum(hn * wr, axis=-1, keepdims=True)
            for j in range(TC // 8):
                rj = r[8 * j:8 * j + 8]
                ij = row8 + (i * TC + 8 * j)
                gt1 = rj > m1
                gt2 = rj > m2
                m2, i2 = (jnp.where(gt1, m1, jnp.where(gt2, rj, m2)),
                          jnp.where(gt1, i1, jnp.where(gt2, ij, i2)))
                m1, i1 = jnp.where(gt1, rj, m1), jnp.where(gt1, ij, i1)

        best = jnp.max(m1, axis=0, keepdims=True)
        ia = jnp.min(jnp.where(m1 == best, i1, S - 1), axis=0, keepdims=True)
        first = jnp.logical_and(m1 == best, i1 == ia)
        mm = jnp.where(first, m2, m1)
        ii = jnp.where(first, i2, i1)
        second = jnp.max(mm, axis=0, keepdims=True)
        ib = jnp.min(jnp.where(mm == second, ii, S - 1), axis=0, keepdims=True)
        ta = jnp.clip(ia[0, 0], 0, S - 1)
        tb = jnp.clip(ib[0, 0], 0, S - 1)

        row16 = lax.broadcasted_iota(I32, (16, D), 0)
        xa = hn_s[pl.ds(ta, 1), :]
        xb = hn_s[pl.ds(tb, 1), :]
        xs = jnp.where(row16 == 0, xa, jnp.where(row16 == 1, xb, 0.0)).astype(BF)
        gte = _dot(xs, wg_v[...])
        up = _dot(xs, wu_v[...])
        act = (gte * jax.nn.sigmoid(gte) * up).astype(BF)
        y = _dot(act, wd_v[...])
        ya = y[0:1] * jax.nn.sigmoid(best)
        yb = y[1:2] * jax.nn.sigmoid(second)

        for i in range(S // TC):
            o_cp(i).wait()
        for t, xr, yr in ((ta, xa, ya), (tb, xb, yb)):
            t0 = pl.multiple_of((t // 16) * 16, 16)
            new = a_s[pl.ds(t, 1), :] + (xr + yr)
            cur = out_v[pl.ds(t0, 16), :].astype(F32)
            out_v[pl.ds(t0, 16), :] = jnp.where(row16 == t - t0, new, cur).astype(BF)

        def fix_cp(t, i):
            t0 = pl.multiple_of((t // 16) * 16, 16)
            return pltpu.make_async_copy(out_v.at[pl.ds(t0, 16)], out_hbm.at[pl.ds(t0, 16)], osem.at[i])

        fix_cp(ta, 0).start()

        @pl.when(ta // 16 != tb // 16)
        def _():
            fix_cp(tb, 1).start()
            fix_cp(tb, 1).wait()

        fix_cp(ta, 0).wait()

    NV = max(8 * NC * G, 8)
    scratch = [
        pltpu.VMEM((S, D), BF), pltpu.VMEM((3, D, D), BF), pltpu.VMEM((D, D), BF), pltpu.VMEM((1, D), BF),
        pltpu.VMEM((D, F), BF), pltpu.VMEM((D, F), BF), pltpu.VMEM((F, D), BF), pltpu.VMEM((S, D), BF),
        pltpu.VMEM((D, D), U32),
        pltpu.VMEM((D, S), F32),
        pltpu.VMEM((D // 2, S), U32),
        pltpu.VMEM((S // 2, D), U32),
        pltpu.VMEM((D // 128, NV, 128), F32),
        pltpu.VMEM((D // 128, S // 2, 128), U32),
        pltpu.VMEM((D, 128), F32),
        pltpu.VMEM((D // 2, S), U32),
        pltpu.VMEM((H, NC * KM // 2, 128), U32),
        [pltpu.VMEM((1, DH, NV, 128), F32) for _ in range(2)],
        pltpu.VMEM((H, DH, S), U32),
        pltpu.VMEM((H, 8, S), F32),
        [pltpu.VMEM((1, DH, 8, W), F32) for _ in range(NQ)],
        pltpu.VMEM((S, D), F32), pltpu.VMEM((S, D), F32),
        pltpu.VMEM((DH, W), F32),
        pltpu.SMEM((2 * NQ * NC,), I32),
        pltpu.SemaphoreType.DMA((12,)), pltpu.SemaphoreType.DMA((S // TC,)),
    ]
    return kernel, scratch


def build(flags=None, **kw):
    kernel, scratch = make_kernel(**kw)

    def fn(A_x, A_wqkv, A_wo, B_x, B_w_r, B_w_gate, B_w_up, B_w_down):
        del B_x
        out = pl.pallas_call(
            kernel,
            grid=(1,),
            in_specs=[pl.BlockSpec(memory_space=pl.ANY)] * 7,
            out_specs=pl.BlockSpec(memory_space=pl.ANY),
            out_shape=jax.ShapeDtypeStruct((S, D), BF),
            scratch_shapes=scratch,
            compiler_params=pltpu.CompilerParams(vmem_limit_bytes=100 * 2 ** 20, flags=flags),
            name="fused_block",
        )(A_x.reshape(S, D), A_wqkv, A_wo, B_w_r.reshape(1, D), B_w_gate, B_w_up, B_w_down)
        return out.reshape(1, S, D)
    return fn


_fused_block = build()


@jax.jit
def pallas_sequential_preLN__mha_block__moe_arch_mod__prompt_kernel(
    A_x: jax.Array,
    A_wqkv: jax.Array,
    A_wo: jax.Array,
    B_x: jax.Array,
    B_w_r: jax.Array,
    B_w_gate: jax.Array,
    B_w_up: jax.Array,
    B_w_down: jax.Array,
):
    return _fused_block(A_x, A_wqkv, A_wo, B_x, B_w_r, B_w_gate, B_w_up, B_w_down)
```

```python
import jax
import jax.numpy as jnp
from jax import lax
import jax.experimental.pallas as pl
import jax.experimental.pallas.tpu as pltpu

S = 2048
D = 512
H = 32
DH = 16
F = 1792
W = 512
CH = 128
NB = CH // 8
NC = S // CH
NQ = S // W
TC = 512
EPS = 1e-5
QSCALE = DH ** -0.5 * 1.4426950408889634
L_MIN = 2.0 ** -50

BF = jnp.bfloat16
F32 = jnp.float32
U32 = jnp.uint32
I32 = jnp.int32


def _pk(x):
    return pltpu.bitcast(x, U32)


def _upk(x):
    return pltpu.bitcast(x, BF)


def _dot(a, b, ca=1, cb=0):
    return lax.dot_general(a, b, (((ca,), (cb,)), ((), ())), preferred_element_type=F32)


def _layernorm(x):
    mu = jnp.sum(x, axis=-1, keepdims=True) * (1.0 / D)
    xc = x - mu
    var = jnp.sum(xc * xc, axis=-1, keepdims=True) * (1.0 / D)
    return xc * lax.rsqrt(var + EPS)


def make_kernel(PAIRS=((3,18),(11,29),(24,34),(39,45),(51,60),(56,66),(71,77),(83,92),(88,98),(108,103),(114,120)), PER=128, NH=1, T3=256, T3D=512,
                SC=False, RD=2, NS=64, MX0=2, CHN=0, KP=(2, 0, 3, 1), ORD=0, AH=2):
    order = [NB * c + NB - 1 - j for c in range(NC) for j in range(NB)]
    vpos = [PER * r + p for r in range(len(order) // PER) for pair in PAIRS for p in pair]
    vpu_blocks = [order[p] for p in vpos]
    mxu_blocks = [b for n, b in enumerate(order) if n not in vpos]
    mo = [MX0 + (sum(b // NB < c for b in mxu_blocks) + 1) // 2 for c in range(NC + 1)]
    vo = [sum(b // NB < c for b in vpu_blocks[::2]) for c in range(NC + 1)]
    mxu_blocks = vpu_blocks[:2 * MX0] + mxu_blocks
    NPAIR = len(vpos) // 2
    kops = [(n, a, d) for d in range(DH) for a in range(4) for n in range(NPAIR) if a < 3 or d < 8]
    kcut = [len(kops) * min(i, NS) // NS for i in range(NQ * NC + 1)]

    def kslot(n, a, d):
        return (4 * n + a) * DH + d // 4 * 4 + KP[d % 4]

    def qslot(u, i, t):
        return 4 * NPAIR * DH + (u * 58 + i) * 2 + t

    def kernel(x_hbm, wqkv_hbm, wo_hbm, wr_hbm, wg_hbm, wu_hbm, wd_hbm, out_hbm,
               x_v, wqkv_v, wo_v, wr_v, wg_v, wu_v, wd_v, out_v,
               wt_s, qt_s, vt_s, xn_s, kv_s, kf_s, kap_s, ot_s,
               ka_s, op_s, qa_s, nu_s, xf_s, hn_s, p_s, o_s, l_s, bad_s, zero_s, zi_s, sem, osem):
        scs = []

        def scope(name):
            if SC:
                if scs:
                    scs.pop().__exit__(None, None, None)
                if name:
                    scs.append(jax.named_scope(name))
                    scs[-1].__enter__()

        x0_cp = pltpu.make_async_copy(x_hbm.at[pl.ds(0, TC)], x_v.at[pl.ds(0, TC)], sem.at[0])
        x1_cp = pltpu.make_async_copy(x_hbm.at[pl.ds(TC, S - TC)], x_v.at[pl.ds(TC, S - TC)], sem.at[1])
        w_cp = [pltpu.make_async_copy(wqkv_hbm.at[:, pl.ds(i * D, D)], wqkv_v.at[i], sem.at[2 + i]) for i in range(3)]
        late = [pltpu.make_async_copy(s_, d_, sem.at[5 + i]) for i, (s_, d_) in enumerate(
            [(wo_hbm, wo_v), (wr_hbm, wr_v), (wg_hbm, wg_v), (wu_hbm, wu_v), (wd_hbm, wd_v)])]

        scope("p1a")
        for c in [x0_cp, w_cp[1], w_cp[0], w_cp[2], x1_cp] + late:
            c.start()
        zero_s[...] = jnp.zeros_like(zero_s)
        p_s[...] = jnp.zeros_like(p_s)
        o_s[...] = jnp.zeros_like(o_s)
        l_s[...] = jnp.ones_like(l_s)
        bad_s[...] = jnp.zeros_like(bad_s)
        for i in range(NH * NQ * NC + 1):
            zi_s[i] = pl.program_id(0)

        def normalize(i):
            x = x_v[pl.ds(i * TC, TC), :].astype(F32)
            xf_s[i * TC:(i + 1) * TC, :] = x
            xn = _layernorm(x).astype(BF)
            xn_s[i * TC // 2:(i + 1) * TC // 2, :] = _pk(xn)
            return xn

        kblk = {}

        def project_k(i, xn, kmax):
            k = _dot(xn, wqkv_v[1])
            kblk.update({i * TC // 8 + b: k[8 * b:8 * b + 8] for b in range(TC // 8)})
            kfp = _pk(k.astype(BF))
            lane = lax.broadcasted_iota(I32, (8, 128), 1)
            for n in range(mo[NC]):
                pair = mxu_blocks[2 * n:2 * n + 2]
                if max(pair) // (TC // 8) != i:
                    continue
                km = _pk(jnp.concatenate([kblk[b] for b in pair], axis=0).astype(BF))
                for g in range(D // 128):
                    kg = km[:, g * 128:(g + 1) * 128]
                    for j in range(4):
                        kr = kg if j == 0 else pltpu.roll(kg, 128 - 2 * DH * j, 1)
                        for e in range(2):
                            ka_s[8 * g + 2 * j + e, 8 * n:8 * n + 8, :] = jnp.where(
                                lane == DH * (1 - e), U32(0x3F803F80), kr)
            for g in range(D // 128):
                for n in range(NPAIR):
                    pair = vpu_blocks[2 * n:2 * n + 2]
                    if max(pair) // (TC // 8) == i:
                        k1, k2 = (kblk[b][:, g * 128:(g + 1) * 128] for b in pair)
                        lo = lane % DH < 8
                        s1 = k2 + pltpu.roll(k2, 120, 1)
                        s2 = s1 - k1
                        s3 = pltpu.roll(k1 - k2, 8, 1)
                        s4 = pltpu.roll(k1, 120, 1) - s2
                        for a, v in enumerate((k1, jnp.where(lo, s1, k2), jnp.where(lo, s2, s3), s4)):
                            kv_s[g, 4 * n + a] = v
                kf_s[g, i * TC // 2:(i + 1) * TC // 2, :] = kfp[:, g * 128:(g + 1) * 128]
            return jnp.maximum(kmax, jnp.max(jnp.abs(k).reshape(TC // 8, 8, D), axis=0))

        def project_qv(i):
            cols = slice(i * TC, (i + 1) * TC)
            qv = _dot(_upk(wt_s[...]), _upk(xn_s[i * TC // 2:(i + 1) * TC // 2, :]), 1, 1)
            qt_s[:, cols] = qv[:D] * QSCALE
            vt_s[:, cols] = _pk(qv[D:].astype(BF))

        def spread_keys(h, slot, dst):
            for n, a, d in kops[kcut[slot]:kcut[slot + 1]]:
                idx = jnp.full((8, 128), DH * (h & 7) + d, I32)
                dst[0, kslot(n, a, d)] = jnp.take_along_axis(kv_s[h >> 3, 4 * n + a], idx, axis=1)

        def put_query(dst, u, i, v):
            for t in range(2):
                dst[0, qslot(u, i, t)] = v[:, t * 128:(t + 1) * 128]

        def put_bound(dst, u, nu):
            put_query(dst, u, 56, nu[:, :W // 2])
            put_query(dst, u, 57, nu[:, W // 2:] - nu[:, :W // 2])

        def spread_queries(terms, u, c, dst):
            for i in range(4 * c, min(4 * c + 4, 56)):
                put_query(dst, u, i, jnp.broadcast_to(terms[i // 8][i % 8:i % 8 + 1], (8, W // 2)))

        def query_terms(q):
            b11, b12, b21, b22 = q[:8, :W // 2], q[:8, W // 2:], q[8:, :W // 2], q[8:, W // 2:]
            t1 = b12 - b11
            t2 = b22 - t1
            return [b11, b21, t2, b22 - b12, b21 - t2, t1, b22]

        def bound(i):
            cols = slice(i * TC, (i + 1) * TC)
            sub = lax.broadcasted_iota(I32, (DH, TC), 0)
            for h in range(H):
                q = qt_s[h * DH:(h + 1) * DH, cols]
                kap = kap_s[h * DH:(h + 1) * DH, :]
                nu = -jnp.sum(jnp.abs(q) * jnp.concatenate([kap] * (TC // 128), axis=1), axis=0, keepdims=True)
                nu = nu.astype(BF).astype(F32)
                nu_s[h, :, cols] = jnp.broadcast_to(nu, (8, TC))
                parts = [q, jnp.where(sub == 0, nu, 0.0)]
                qa_s[h, :, cols] = _pk(jnp.concatenate(parts[::1 - 2 * (h % 2)], axis=0).astype(BF))
                if h < NH:
                    put_bound(op_s[h], i, jnp.broadcast_to(nu, (8, TC)))
                    for c in range(NC):
                        spread_queries(query_terms(q), i, c, op_s[h])

        x0_cp.wait()
        xn = normalize(0)
        w_cp[1].wait()
        kmax = project_k(0, xn, jnp.zeros((8, D), F32))
        w_cp[0].wait()
        w_cp[2].wait()
        scope("p1b")
        wt_s[0:D // 2, :] = _pk(wqkv_v[0].T)
        wt_s[D // 2:D, :] = _pk(wqkv_v[2].T)
        x1_cp.wait() if ORD else None
        project_qv(0)
        None if ORD else x1_cp.wait()
        for i in range(1, S // TC):
            kmax = project_k(i, normalize(i), kmax)
        kmax = jnp.max(kmax, axis=0, keepdims=True)
        for g in range(D // 128):
            kap_s[g * 128:(g + 1) * 128, :] = jnp.broadcast_to(kmax[:, g * 128:(g + 1) * 128], (128, 128)).T
        for slot in range(NQ * NC):
            for h in range(NH):
                spread_keys(h, slot, op_s[h])
        for i in range(1, S // TC):
            bound(i - 1)
            project_qv(i)
        bound(S // TC - 1)

        scope("p2")

        def back(h, u, c, p, o, l, bad):
            vc = vt_s[pl.ds(pl.multiple_of(jnp.maximum(h, 0) * 8, 8), 8), c * CH:(c + 1) * CH]
            o = o + _dot(_upk(vc), p)
            if c == NC - 1:
                l = jnp.sum(l, axis=0, keepdims=True)
                bad = jnp.where(l >= L_MIN, bad, 1.0)
                ot_s[pl.ds(pl.multiple_of(h * 8 + 8, 8), 8), u * W:(u + 1) * W] = _pk((o * (1.0 / l)).astype(BF))
            return o, bad

        def heads(hh, par):
            st = {}
            z0 = pltpu.bitcast(zero_s[0:8, 0:128], I32)[0, 0]

            def front(e, u, c, l):
                h = hh * NH + e
                n = (e * NQ + u) * NC + c
                z = zi_s[n] + z0
                cols = slice(u * W, (u + 1) * W)

                def score(e, u, m0, m1):
                    s = _dot(_upk(ka_s[hh * NH + e, 8 * m0:8 * m1, 0:2 * DH]),
                             _upk(qa_s[hh * NH + e, :, u * W:(u + 1) * W]))
                    for j, b in enumerate(mxu_blocks[2 * m0:2 * m1]):
                        st["s", e, u, b] = s[8 * j:8 * j + 8]

                score(e, u, 0 if n == 0 else mo[c] + AH, min(mo[c + 1] + AH, mo[NC]))
                if AH and c == NC - 1 and n + 1 < NH * NQ * NC:
                    score(e + (u + 1) // NQ, (u + 1) % NQ, mo[0] if u + 1 < NQ else 0, mo[0] + AH)
                src, dst = op_s[par * NH + e], op_s[(1 - par) * NH + e]
                hq = jnp.minimum(h + NH, H - 1)
                if ("p", n - RD) in st:
                    dst[z, qslot(NQ, 0, 0)] = st["p", n - RD]
                if c == 0:
                    st["q"] = query_terms(qt_s[pl.ds(pl.multiple_of(hq * DH, DH), DH), cols])
                    put_bound(dst, u, nu_s[hq, :, cols])
                spread_keys(hq, u * NC + c, dst)
                spread_queries(st["q"], u, c, dst)
                for j in range(max(vo[c], MX0 if u == 0 else 0), vo[c + 1]):
                    zz = z + zi_s[NH * NQ * NC] if j > vo[c] else z

                    def query(i):
                        return jnp.concatenate([src[zz, qslot(u, i, t)] for t in range(2)], axis=1)

                    def term(m, a, d0, acc):
                        tot = acc if CHN else None
                        for d in range(8):
                            kd = src[zz, kslot(j, a, d0 + d)]
                            t = jnp.concatenate([kd] * (W // 256), axis=1) * query(8 * m + d)
                            tot = t if tot is None else tot + t
                        return tot if CHN else tot + acc

                    m1 = term(0, 0, 0, query(56))
                    c11 = term(1, 0, 8, m1)
                    u2 = term(2, 2, 0, m1)
                    m5 = term(5, 1, 0, query(57))
                    c12 = term(6, 3, 0, u2 + m5)
                    u3 = term(3, 2, 8, u2)
                    c21 = term(4, 1, 8, u3)
                    st["s", e, u, vpu_blocks[2 * j]] = jnp.concatenate([c11, c12], axis=1)
                    st["s", e, u, vpu_blocks[2 * j + 1]] = jnp.concatenate([c21, u3 + m5], axis=1)
                p = {b: jnp.exp2(st.pop(("s", e, u, NB * c + b))) for b in range(NB - 1, -1, -1)}
                st["p", n] = p[NB - 1][:, :128]
                for b in range(NB - 1, -1, -1):
                    l = p[b] if l is None else l + p[b]
                return jnp.concatenate([p[b] for b in range(NB)], axis=0), l

            pend, o, l, bad = (hh * NH - 1, NQ - 1, NC - 1, p_s[...]), o_s[...], l_s[...], bad_s[...]
            for e in range(NH):
                for u in range(NQ):
                    for c in range(NC):
                        p, l_new = front(e, u, c, l if c else None)
                        o, bad = back(*pend, o, l, bad)
                        if c == 0:
                            o = zero_s[...]
                        pend, l = (hh * NH + e, u, c, p), l_new
            p_s[...] = p
            o_s[...] = o
            l_s[...] = l
            bad_s[...] = bad

        def step(hh, carry):
            for par in range(2):
                pl.when(hh % 2 == par)(lambda: heads(hh, par))
            return carry

        lax.fori_loop(0, H // NH, step, 0)
        _, bad = back(H - 1, NQ - 1, NC - 1, p_s[...], o_s[...], l_s[...], bad_s[...])

        scope("chk")

        @pl.when(jnp.max(bad) > 0.0)
        def _exact():
            def body(t, carry):
                h = t // (S // 128)
                q0 = pl.multiple_of((t % (S // 128)) * 128, 128)
                g = h // 8
                qg = qt_s[pl.ds(pl.multiple_of(g * 128, 128), 128), pl.ds(q0, 128)]
                rows = lax.broadcasted_iota(I32, (128, 128), 0) // DH
                qg = jnp.where(rows == h % 8, qg, 0.0).astype(BF)
                kg = _upk(kf_s[g])
                lanes = lax.broadcasted_iota(I32, kg.shape, 1) // DH
                kg = jnp.where(lanes == h % 8, kg, jnp.zeros_like(kg))
                s = _dot(kg, qg)
                p = jnp.exp2(s - jnp.max(s, axis=0, keepdims=True))
                l = jnp.sum(p, axis=0, keepdims=True)
                o = _dot(_upk(vt_s[pl.ds(pl.multiple_of(h * 8, 8), 8), :]), p.astype(BF))
                ot_s[pl.ds(pl.multiple_of(h * 8 + 8, 8), 8), pl.ds(q0, 128)] = _pk((o * (1.0 / l)).astype(BF))
                return carry
            lax.fori_loop(0, H * (S // 128), body, 0)

        scope("p3")
        for c in late:
            c.wait()
        wr = wr_v[...].reshape(1, D).astype(F32)
        lane = lax.broadcasted_iota(I32, (8, 128), 1)
        rs = [jnp.zeros((8, 128), F32)] * (S // 1024)

        def o_cp(i):
            return pltpu.make_async_copy(out_v.at[pl.ds(i * T3D, T3D)], out_hbm.at[pl.ds(i * T3D, T3D)], osem.at[i])

        att_next = _dot(_upk(ot_s[8:, 0:T3]), wo_v[...], 0, 0)
        for i in range(S // T3):
            rows = slice(i * T3, (i + 1) * T3)
            att = att_next
            if i + 1 < S // T3:
                att_next = _dot(_upk(ot_s[8:, (i + 1) * T3:(i + 2) * T3]), wo_v[...], 0, 0)
            h1 = xf_s[rows, :] + att
            hn = _layernorm(h1)
            hn_s[rows, :] = hn
            out_v[rows, :] = (h1 + hn).astype(BF)
            if (i + 1) * T3 % T3D == 0:
                o_cp((i + 1) * T3 // T3D - 1).start()
            r = jnp.sum(hn * wr, axis=-1, keepdims=True)
            for j in range(T3 // 8):
                n = i * T3 // 8 + j
                rs[n // 128] = jnp.where(lane == n % 128, r[8 * j:8 * j + 8], rs[n // 128])

        scope("ffn")
        r = jnp.concatenate(rs, axis=1)
        tok = (8 * lax.broadcasted_iota(I32, r.shape, 1) + lax.broadcasted_iota(I32, r.shape, 0)).astype(F32)

        def top(r):
            m = jnp.max(jnp.max(r, axis=1, keepdims=True), axis=0, keepdims=True)
            t = jnp.min(jnp.min(jnp.where(r == m, tok, S - 1.0), axis=1, keepdims=True), axis=0, keepdims=True)
            return m, t

        ra, fa = top(r)
        rb, fb = top(jnp.where(tok == fa, -jnp.inf, r))
        ta = jnp.clip(fa.astype(I32)[0, 0], 0, S - 1)
        tb = jnp.clip(fb.astype(I32)[0, 0], 0, S - 1)

        row16 = lax.broadcasted_iota(I32, (16, D), 0)
        xs = jnp.where(row16 == 0, hn_s[pl.ds(ta, 1), :], jnp.where(row16 == 1, hn_s[pl.ds(tb, 1), :], 0.0))
        xs = xs.astype(BF)
        gate = _dot(xs, wg_v[...])
        act = (gate * jax.nn.sigmoid(gate) * _dot(xs, wu_v[...])).astype(BF)
        y = _dot(act, wd_v[...])

        scope("fix")
        for i in range(S // T3D):
            o_cp(i).wait()
        for t, yr in ((ta, y[0:1] * jax.nn.sigmoid(ra)), (tb, y[1:2] * jax.nn.sigmoid(rb))):
            t0 = pl.multiple_of((t // 16) * 16, 16)
            cur = out_v[pl.ds(t0, 16), :].astype(F32)
            out_v[pl.ds(t0, 16), :] = jnp.where(row16 == t - t0, cur + yr, cur).astype(BF)

        def fix_cp(t, i):
            t0 = pl.multiple_of((t // 16) * 16, 16)
            return pltpu.make_async_copy(out_v.at[pl.ds(t0, 16)], out_hbm.at[pl.ds(t0, 16)], osem.at[i])

        fix_cp(ta, 0).start()

        @pl.when(ta // 16 != tb // 16)
        def _():
            fix_cp(tb, 1).start()
            fix_cp(tb, 1).wait()

        fix_cp(ta, 0).wait()
        scope(None)

    scratch = [
        pltpu.VMEM((S, D), BF), pltpu.VMEM((3, D, D), BF), pltpu.VMEM((D, D), BF), pltpu.VMEM((D,), BF),
        pltpu.VMEM((D, F), BF), pltpu.VMEM((D, F), BF), pltpu.VMEM((F, D), BF), pltpu.VMEM((S, D), BF),
        pltpu.VMEM((D, D), U32),
        pltpu.VMEM((D, S), F32),
        pltpu.VMEM((D // 2, S), U32),
        pltpu.VMEM((S // 2, D), U32),
        pltpu.VMEM((D // 128, 4 * NPAIR, 8, 128), F32),
        pltpu.VMEM((D // 128, S // 2, 128), U32),
        pltpu.VMEM((D, 128), F32),
        pltpu.VMEM((D // 2 + 8, S), U32),
        pltpu.VMEM((H, 8 * mo[NC], 128), U32),
        [pltpu.VMEM((1, qslot(NQ, 2, 0), 8, 128), F32) for _ in range(2 * NH)],
        pltpu.VMEM((H, DH, S), U32),
        pltpu.VMEM((H, 8, S), F32),
        pltpu.VMEM((S, D), F32), pltpu.VMEM((S, D), F32),
        pltpu.VMEM((CH, W), F32), pltpu.VMEM((DH, W), F32), pltpu.VMEM((8, W), F32), pltpu.VMEM((1, W), F32),
        pltpu.VMEM((DH, W), F32),
        pltpu.SMEM((NH * NQ * NC + 1,), I32),
        pltpu.SemaphoreType.DMA((10,)), pltpu.SemaphoreType.DMA((S // T3D,)),
    ]
    return kernel, scratch


def build(flags=None, **kw):
    kernel, scratch = make_kernel(**kw)

    def fn(A_x, A_wqkv, A_wo, B_x, B_w_r, B_w_gate, B_w_up, B_w_down):
        del B_x
        out = pl.pallas_call(
            kernel,
            grid=(1,),
            in_specs=[pl.BlockSpec(memory_space=pl.ANY)] * 7,
            out_specs=pl.BlockSpec(memory_space=pl.ANY),
            out_shape=jax.ShapeDtypeStruct((S, D), BF),
            scratch_shapes=scratch,
            compiler_params=pltpu.CompilerParams(vmem_limit_bytes=120 * 2 ** 20, flags=flags),
            name="fused_block",
        )(A_x.reshape(S, D), A_wqkv, A_wo, B_w_r, B_w_gate, B_w_up, B_w_down)
        return out.reshape(1, S, D)
    return fn


_fused_block = build(KP=(0,1,2,3))


@jax.jit
def pallas_sequential_preLN__mha_block__moe_arch_mod__prompt_kernel(
    A_x: jax.Array,
    A_wqkv: jax.Array,
    A_wo: jax.Array,
    B_x: jax.Array,
    B_w_r: jax.Array,
    B_w_gate: jax.Array,
    B_w_up: jax.Array,
    B_w_down: jax.Array,
):
    return _fused_block(A_x, A_wqkv, A_wo, B_x, B_w_r, B_w_gate, B_w_up, B_w_down)
```

```python
import jax
import jax.numpy as jnp
from jax import lax
import jax.experimental.pallas as pl
import jax.experimental.pallas.tpu as pltpu

S = 2048
D = 512
H = 32
DH = 16
F = 1792
EPS = 1e-5
QSCALE = DH ** -0.5 * 1.4426950408889634
L_MIN = 2.0 ** -64

W = 512
CH = 128
NB = CH // 8
NC = S // CH
NQ = S // W
TC = 512
TM = 128
TO = 128
OUT_CUTS = (0, 1152, 1792, 2048)

BF = jnp.bfloat16
F32 = jnp.float32
U32 = jnp.uint32
I32 = jnp.int32

VPU_PAIRS = tuple((a + r, b + r) for r in (0, 128) for a, b in (
    (3, 18), (11, 29), (24, 34), (39, 45), (51, 60), (56, 66), (71, 77), (83, 92), (88, 98),
    (108, 103), (114, 120)))


def _pk(x):
    return pltpu.bitcast(x, U32)


def _upk(x):
    return pltpu.bitcast(x, BF)


def _dot(a, b, ca=1, cb=0):
    return lax.dot_general(a, b, (((ca,), (cb,)), ((), ())), preferred_element_type=F32)


def _center(x):
    xc = x - jnp.sum(x, axis=-1, keepdims=True) * (1.0 / D)
    return xc, lax.rsqrt(jnp.sum(xc * xc, axis=-1, keepdims=True) * (1.0 / D) + EPS)


def build(vpu_pairs=VPU_PAIRS, l_min=L_MIN):
    order = [NB * c + NB - 1 - j for c in range(NC) for j in range(NB)]
    vpu_blocks = [order[p] for pair in vpu_pairs for p in pair]
    mxu_blocks = [b for b in order if b not in vpu_blocks]
    mo = [1 + (sum(b // NB < c for b in mxu_blocks) + 1) // 2 for c in range(NC + 1)]
    vo = [sum(b // NB < c for b in vpu_blocks[::2]) for c in range(NC + 1)]
    mxu_blocks = vpu_blocks[:2] + mxu_blocks
    npair = len(vpu_pairs)
    key_ops = [(n, a, d) for d in range(DH) for a in range(4) for n in range(npair) if a < 3 or d < 8]
    key_cut = [len(key_ops) * i // (NQ * NC) for i in range(NQ * NC + 1)]

    def kslot(n, a, d):
        return (4 * n + a) * DH + d // 4 * 4 + (2, 0, 3, 1)[d % 4]

    def qslot(u, i, t):
        return 4 * npair * DH + (u * 58 + i) * 2 + t

    def kernel(x_hbm, wqkv_hbm, wo_hbm, wr_hbm, wg_hbm, wu_hbm, wd_hbm, out_hbm,
               x_v, wqkv_v, wo_v, wg_v, wu_v, wd_v, out_v,
               wt_s, qt_s, vt_s, xn_s, kv_s, kmax_s, ot_s, ka_s, op_s, qa_s, nu_s, xf_s, hn_s,
               p_s, o_s, inv_s, zero_s, bad_s, wr_v, izero_s, sem, osem):
        def x_rows(i, r0, r1):
            rows = pl.ds(r0, r1 - r0)
            return pltpu.make_async_copy(x_hbm.at[rows], x_v.at[rows], sem.at[i])

        x_cp = [x_rows(0, 0, TC), x_rows(1, TC, 2 * TC), x_rows(2, 2 * TC, S)]
        w_cp = [pltpu.make_async_copy(wqkv_hbm.at[:, pl.ds(i * D, D)], wqkv_v.at[i], sem.at[3 + i])
                for i in range(3)]
        late = [pltpu.make_async_copy(src, dst, sem.at[6 + i]) for i, (src, dst) in enumerate(
            [(wo_hbm, wo_v), (wr_hbm, wr_v), (wg_hbm, wg_v), (wu_hbm, wu_v), (wd_hbm, wd_v)])]
        for cp in [x_cp[0], w_cp[1], w_cp[0], x_cp[1], w_cp[2], x_cp[2]] + late:
            cp.start()
        zero_s[...] = jnp.zeros_like(zero_s)
        p_s[...] = jnp.zeros_like(p_s)
        o_s[...] = jnp.zeros_like(o_s)
        inv_s[...] = jnp.ones_like(inv_s)
        bad_s[...] = jnp.zeros_like(bad_s)
        for i in range(izero_s.shape[0]):
            izero_s[i] = pl.program_id(0)

        def normalize(i):
            x = x_v[i * TC:(i + 1) * TC, :].astype(F32)
            xf_s[i * TC:(i + 1) * TC, :] = x
            xc, rstd = _center(x)
            xn = (xc * rstd).astype(BF)
            xn_s[i * TC // 2:(i + 1) * TC // 2, :] = _pk(xn)
            return xn

        kblk = {}

        def arrange_keys(i, k, kmax):
            kblk.update({i * TC // 8 + b: k[8 * b:8 * b + 8] for b in range(TC // 8)})
            lane = lax.broadcasted_iota(I32, (8, 128), 1)
            for n in range(mo[NC]):
                pair = mxu_blocks[2 * n:2 * n + 2]
                if max(pair) // (TC // 8) != i:
                    continue
                km = _pk(jnp.concatenate([kblk[b] for b in pair], axis=0).astype(BF))
                for g in range(D // 128):
                    kg = km[:, g * 128:(g + 1) * 128]
                    for j in range(4):
                        kr = kg if j == 0 else pltpu.roll(kg, 128 - 2 * DH * j, 1)
                        for e in range(2):
                            ka_s[8 * g + 2 * j + e, 8 * n:8 * n + 8, :] = jnp.where(
                                lane == DH * (1 - e), U32(0x3F803F80), kr)
            for g in range(D // 128):
                for n in range(npair):
                    pair = vpu_blocks[2 * n:2 * n + 2]
                    if max(pair) // (TC // 8) != i:
                        continue
                    k1, k2 = (kblk[b][:, g * 128:(g + 1) * 128] for b in pair)
                    lo = lane % DH < 8
                    s1 = k2 + pltpu.roll(k2, 120, 1)
                    s2 = s1 - k1
                    s3 = pltpu.roll(k1 - k2, 8, 1)
                    s4 = pltpu.roll(k1, 120, 1) - s2
                    for a, v in enumerate((k1, jnp.where(lo, s1, k2), jnp.where(lo, s2, s3), s4)):
                        kv_s[g, 4 * n + a] = v
            return jnp.maximum(kmax, jnp.max(jnp.abs(k).reshape(TC // 8, 8, D), axis=0))

        def project_t(i, part, jobs=()):
            cols = slice(i * TC, (i + 1) * TC)
            marks = []
            for r in range(0, D, TM):
                y = None
                for k in range(0, D, 128):
                    t = _dot(_upk(wt_s[part, r // 2:(r + TM) // 2, k:k + 128]),
                             _upk(xn_s[i * TC // 2:(i + 1) * TC // 2, k:k + 128]), 1, 1)
                    y = t if y is None else y + t
                    marks += [y[j:j + 8, :128] for j in range(0, TM, 8)]
                if part == 0:
                    qt_s[r:r + TM, cols] = y * QSCALE
                else:
                    vt_s[r // 2:(r + TM) // 2, cols] = _pk(y.astype(BF))
            for j, job in enumerate(jobs):
                spare = pl.ds(pl.multiple_of(izero_s[0] + D, 8), 8)
                kmax_s[spare, :] = marks[j * len(marks) // len(jobs)]
                bound(*job)

        def spread_keys(h, slot, dst):
            for n, a, d in key_ops[key_cut[slot]:key_cut[slot + 1]]:
                idx = jnp.full((8, 128), DH * (h & 7) + d, I32)
                dst[0, kslot(n, a, d)] = jnp.take_along_axis(
                    kv_s[h >> 3, 4 * n + a], idx, axis=1, mode="promise_in_bounds")

        def put_query(dst, u, i, v):
            for t in range(2):
                dst[0, qslot(u, i, t)] = v[:, t * 128:(t + 1) * 128]

        def query_terms(q):
            b11, b12, b21, b22 = q[:8, :W // 2], q[:8, W // 2:], q[8:, :W // 2], q[8:, W // 2:]
            t1 = b12 - b11
            t2 = b22 - t1
            return [b11, b21, t2, b22 - b12, b21 - t2, t1, b22]

        def spread_queries(terms, u, c, dst):
            for i in range(4 * c, min(4 * c + 4, 56)):
                put_query(dst, u, i, jnp.broadcast_to(terms[i // 8][i % 8:i % 8 + 1], (8, W // 2)))

        def bound(u, h):
            cols = slice(u * W, (u + 1) * W)
            q = qt_s[h * DH:(h + 1) * DH, cols]
            kmax = kmax_s[h * DH:(h + 1) * DH, :]
            top = jnp.sum(jnp.abs(q) * jnp.concatenate([kmax] * (W // 128), axis=1), axis=0, keepdims=True)
            top = jnp.broadcast_to(jnp.maximum(top[:, :W // 2], top[:, W // 2:]), (8, W // 2))
            bits = (pltpu.bitcast(top, U32) >> 16) | U32(0x8000)
            nu = pltpu.bitcast(bits << 16, F32)
            nu_s[h, u] = nu
            row = jnp.where(lax.broadcasted_iota(I32, (8, W // 2), 0) == 0, bits, U32(0))
            qa_s[h, 8 * (h % 2):8 * (h % 2) + 8, cols] = _pk(q.astype(BF))
            qa_s[h, 8 - 8 * (h % 2):16 - 8 * (h % 2), cols] = jnp.concatenate([row, row], axis=1)
            if h == 0:
                put_query(op_s[0], u, 56, nu)
                for c in range(NC):
                    spread_queries(query_terms(q), u, c, op_s[0])

        x_cp[0].wait()
        xn = normalize(0)
        w_cp[1].wait()
        k = _dot(xn, wqkv_v[1])
        w_cp[0].wait()
        x_cp[1].wait()
        wt_s[0] = _pk(wqkv_v[0].T)
        project_t(0, 0)
        kmax = arrange_keys(0, k, jnp.zeros((8, D), F32))
        k = _dot(normalize(1), wqkv_v[1])
        w_cp[2].wait()
        x_cp[2].wait()
        project_t(1, 0)
        kmax = arrange_keys(1, k, kmax)
        wt_s[1] = _pk(wqkv_v[2].T)
        k = _dot(normalize(2), wqkv_v[1])
        project_t(0, 1)
        kmax = arrange_keys(2, k, kmax)
        k = _dot(normalize(3), wqkv_v[1])
        project_t(1, 1)
        kmax = arrange_keys(3, k, kmax)
        kmax = jnp.max(kmax, axis=0, keepdims=True)
        for g in range(D // 128):
            kmax_s[g * 128:(g + 1) * 128, :] = jnp.broadcast_to(kmax[:, g * 128:(g + 1) * 128], (128, 128)).T
        jobs = [(u, h) for u in range(NQ) for h in range(H)]
        job_cut = (0, 20, 56, 92, 128)
        for i, (chunk, part) in enumerate(((2, 0), (3, 0), (2, 1), (3, 1))):
            for slot in range(i * NC, (i + 1) * NC):
                spread_keys(0, slot, op_s[0])
            project_t(chunk, part, jobs[job_cut[i]:job_cut[i + 1]])
        for cp in late:
            cp.wait()

        def weigh_values(h, u, c, p, o, inv):
            vc = vt_s[pl.ds(pl.multiple_of(jnp.maximum(h, 0) * 8, 8), 8), c * CH:(c + 1) * CH]
            o = o + _dot(_upk(vc), p)
            if c == NC - 1:
                out = o * jnp.concatenate([inv, inv], axis=0)
                ot_s[pl.ds(pl.multiple_of(h * 8 + 8, 8), 8), u * W:(u + 1) * W] = _pk(out.astype(BF))
            return o

        def head(h, src, dst):
            score, first_p = {}, {}
            z0 = pltpu.bitcast(zero_s[0:8, 0:128], I32)[0, 0]

            def mxu_scores(u, m0, m1):
                s = _dot(_upk(ka_s[h, 8 * m0:8 * m1, 0:2 * DH]), _upk(qa_s[h, :, u * W:(u + 1) * W]))
                for j, b in enumerate(mxu_blocks[2 * m0:2 * m1]):
                    score[u, b] = s[8 * j:8 * j + 8]

            def vpu_scores(u, j, z):
                def query(i):
                    return jnp.concatenate([src[z, qslot(u, i, t)] for t in range(2)], axis=1)

                def term(m, a, d0):
                    tot = None
                    for d in range(8):
                        t = jnp.concatenate([src[z, kslot(j, a, d0 + d)]] * 2, axis=1) * query(8 * m + d)
                        tot = t if tot is None else tot + t
                    return tot

                m1 = term(0, 0, 0) + query(56)
                c11 = term(1, 0, 8) + m1
                u2 = term(2, 2, 0) + m1
                m5 = term(5, 1, 0)
                c12 = term(6, 3, 0) + (u2 + m5)
                u3 = term(3, 2, 8) + u2
                c21 = term(4, 1, 8) + u3
                score[u, vpu_blocks[2 * j]] = jnp.concatenate([c11, c12], axis=1)
                score[u, vpu_blocks[2 * j + 1]] = jnp.concatenate([c21, u3 + m5], axis=1)

            def probabilities(u, c, l, terms):
                n = u * NC + c
                z = izero_s[n] + z0
                mxu_scores(u, mo[c] + 1 if n else 0, min(mo[c + 1] + 1, mo[NC]))
                if c == NC - 1 and u + 1 < NQ:
                    mxu_scores(u + 1, mo[0], mo[0] + 1)
                hn = jnp.minimum(h + 1, H - 1)
                if n >= 2:
                    dst[z, qslot(NQ, 0, 0)] = first_p[n - 2]
                if c == 0:
                    terms = query_terms(qt_s[pl.ds(pl.multiple_of(hn * DH, DH), DH), u * W:(u + 1) * W])
                    put_query(dst, u, 56, nu_s[hn, u])
                spread_keys(hn, n, dst)
                spread_queries(terms, u, c, dst)
                for j in range(max(vo[c], 1 if u == 0 else 0), vo[c + 1]):
                    vpu_scores(u, j, z + izero_s[NQ * NC + j - vo[c] - 1] if j > vo[c] else z)
                p = {b: jnp.exp2(score.pop((u, NB * c + b))) for b in range(NB - 1, -1, -1)}
                first_p[n] = p[NB - 1][:, :128]
                for b in range(NB - 1, -1, -1):
                    l = p[b] if l is None else l + p[b]
                return jnp.concatenate([p[b] for b in range(NB)], axis=0), l, terms

            pending, o, l, bad = (h - 1, NQ - 1, NC - 1, p_s[...]), o_s[...], inv_s[...], bad_s[...]
            terms = None
            for u in range(NQ):
                for c in range(NC):
                    p, l_new, terms = probabilities(u, c, l if c else None, terms)
                    o = weigh_values(*pending, o, l)
                    if c == 0:
                        o = zero_s[...]
                    if c == NC - 1:
                        tot = jnp.broadcast_to(jnp.sum(l_new, axis=0, keepdims=True), (8, W))
                        for t in range(0, W, 128):
                            bad = jnp.where(tot[:, t:t + 128] >= l_min, bad, 1.0)
                        l_new = pltpu.reciprocal(tot, approx=True)
                        l_new = l_new * (2.0 - tot * l_new)
                    pending, l = (h, u, c, p), l_new
            p_s[...] = p
            o_s[...] = o
            inv_s[...] = l
            bad_s[...] = bad

        def two_heads(i, carry):
            head(2 * i, op_s[0], op_s[1])
            pl.when(izero_s[0] == 0)(lambda: head(2 * i + 1, op_s[1], op_s[0]))
            return carry

        lax.fori_loop(0, H // 2, two_heads, 0)

        @pl.when(jnp.max(bad_s[...]) > 0.0)
        def _with_true_maximum():
            def tile(t, carry):
                h = t // (S // 128)
                c0 = pl.multiple_of((h // 8) * 128, 128)
                q0 = pl.multiple_of((t % (S // 128)) * 128, 128)

                @pl.when(t % (8 * S // 128) == 0)
                def _():
                    @pl.loop(0, S // 128)
                    def _(r):
                        xn = _upk(xn_s[pl.ds(pl.multiple_of(r * 64, 64), 64), :])
                        rows = pl.ds(pl.multiple_of(r * 128, 128), 128)
                        hn_s[rows, 0:128] = _dot(xn, wqkv_v[1, :, pl.ds(c0, 128)])

                rows = lax.broadcasted_iota(I32, (128, 128), 0) // DH
                lanes = lax.broadcasted_iota(I32, (S, 128), 1) // DH
                qh = jnp.where(rows == h % 8, qt_s[pl.ds(c0, 128), pl.ds(q0, 128)], 0.0)
                kh = jnp.where(lanes == h % 8, hn_s[:, 0:128], 0.0)
                s = _dot(kh.astype(BF), qh.astype(BF))
                p = jnp.exp2(s - jnp.max(s, axis=0, keepdims=True))
                r8 = pl.multiple_of(h * 8, 8)
                o = _dot(_upk(vt_s[pl.ds(r8, 8), :]), p.astype(BF))
                o = o * (1.0 / jnp.sum(p, axis=0, keepdims=True))
                ot_s[pl.ds(r8 + 8, 8), pl.ds(q0, 128)] = _pk(o.astype(BF))
                o_s[:, pl.ds(pl.multiple_of(q0 % W, 128), 128)] = o
                return carry

            lax.fori_loop(0, H * (S // 128), tile, 0)
            p_s[...] = jnp.zeros_like(p_s)
            inv_s[...] = jnp.ones_like(inv_s)

        def out_cp(i):
            rows = pl.ds(OUT_CUTS[i], OUT_CUTS[i + 1] - OUT_CUTS[i])
            return pltpu.make_async_copy(out_v.at[rows], out_hbm.at[rows], osem.at[i])

        def attended(i):
            return _dot(_upk(ot_s[8:, i * TO:(i + 1) * TO]), wo_v[...], 0, 0)

        wr = wr_v[...].reshape(1, D).astype(F32)
        m1 = m2 = jnp.full((8, 1), -jnp.inf, F32)
        i1 = i2 = jnp.full((8, 1), -1, I32)
        att_next = attended(0)
        weigh_values(H - 1, NQ - 1, NC - 1, p_s[...], o_s[...], inv_s[...])
        for i in range(S // TO):
            rows = slice(i * TO, (i + 1) * TO)
            att = att_next
            if i + 1 < S // TO:
                att_next = attended(i + 1)
            h1 = xf_s[rows, :] + att
            hc, rstd = _center(h1)
            hn = hc * rstd
            hn_s[rows, :] = hn
            out_v[rows, :] = (h1 + hn).astype(BF)
            r = jnp.sum(hc * wr, axis=-1, keepdims=True) * rstd
            for j in range(TO // 8):
                n = i * TO // 8 + j
                rj = r[8 * j:8 * j + 8]
                gt1, gt2 = rj > m1, rj > m2
                m2, i2 = jnp.where(gt1, m1, jnp.where(gt2, rj, m2)), jnp.where(gt1, i1, jnp.where(gt2, n, i2))
                m1, i1 = jnp.where(gt1, rj, m1), jnp.where(gt1, n, i1)
            if (i + 1) * TO in OUT_CUTS:
                out_cp(OUT_CUTS.index((i + 1) * TO) - 1).start()

        sub = lax.broadcasted_iota(I32, (8, 1), 0)
        i1, i2 = (8 * i1 + sub).astype(F32), (8 * i2 + sub).astype(F32)

        def top(r, tok):
            m = jnp.max(r, axis=0, keepdims=True)
            return m, jnp.min(jnp.where(r == m, tok, S - 1.0), axis=0, keepdims=True)

        ra, fa = top(m1, i1)
        rb, fb = top(jnp.where(i1 == fa, m2, m1), jnp.where(i1 == fa, i2, i1))
        ta = jnp.clip(fa.astype(I32)[0, 0], 0, S - 1)
        tb = jnp.clip(fb.astype(I32)[0, 0], 0, S - 1)

        row16 = lax.broadcasted_iota(I32, (16, D), 0)
        xs = jnp.where(row16 == 0, hn_s[pl.ds(ta, 1), :], jnp.where(row16 == 1, hn_s[pl.ds(tb, 1), :], 0.0))
        xs = xs.astype(BF)
        gate = _dot(xs, wg_v[...])
        act = (gate * jax.nn.sigmoid(gate) * _dot(xs, wu_v[...])).astype(BF)
        y = _dot(act, wd_v[...])

        def tile_of(t):
            return pl.ds(pl.multiple_of((t // 16) * 16, 16), 16)

        for i in range(len(OUT_CUTS) - 1):
            out_cp(i).wait()
        for t, yr in ((ta, y[0:1] * jax.nn.sigmoid(ra)), (tb, y[1:2] * jax.nn.sigmoid(rb))):
            cur = out_v[tile_of(t), :].astype(F32)
            out_v[tile_of(t), :] = jnp.where(row16 == t % 16, cur + yr, cur).astype(BF)

        def fix_cp(t, i):
            return pltpu.make_async_copy(out_v.at[tile_of(t)], out_hbm.at[tile_of(t)], osem.at[i])

        fix_cp(ta, 0).start()

        @pl.when(ta // 16 != tb // 16)
        def _():
            fix_cp(tb, 1).start()
            fix_cp(tb, 1).wait()

        fix_cp(ta, 0).wait()

    scratch = [
        pltpu.VMEM((S, D), BF), pltpu.VMEM((3, D, D), BF), pltpu.VMEM((D, D), BF),
        pltpu.VMEM((D, F), BF), pltpu.VMEM((D, F), BF), pltpu.VMEM((F, D), BF), pltpu.VMEM((S, D), BF),
        pltpu.VMEM((2, D // 2, D), U32),
        pltpu.VMEM((D, S), F32),
        pltpu.VMEM((D // 2, S), U32),
        pltpu.VMEM((S // 2, D), U32),
        pltpu.VMEM((D // 128, 4 * npair, 8, 128), F32),
        pltpu.VMEM((D + 32, 128), F32),
        pltpu.VMEM((D // 2 + 8, S), U32),
        pltpu.VMEM((H, 32 * pl.cdiv(mo[NC], 4), 128), U32),
        [pltpu.VMEM((1, qslot(NQ, 2, 0), 8, 128), F32) for _ in range(2)],
        pltpu.VMEM((H, DH, S), U32),
        pltpu.VMEM((H, NQ, 8, W // 2), F32),
        pltpu.VMEM((S, D), F32), pltpu.VMEM((S, D), F32),
        pltpu.VMEM((CH, W), F32), pltpu.VMEM((DH, W), F32), pltpu.VMEM((8, W), F32),
        pltpu.VMEM((DH, W), F32), pltpu.VMEM((8, 128), F32), pltpu.VMEM((D,), BF),
        pltpu.SMEM((NQ * NC + 8,), I32),
        pltpu.SemaphoreType.DMA((11,)), pltpu.SemaphoreType.DMA((len(OUT_CUTS) - 1,)),
    ]

    def fused_block(A_x, A_wqkv, A_wo, B_x, B_w_r, B_w_gate, B_w_up, B_w_down):
        del B_x
        out = pl.pallas_call(
            kernel,
            grid=(1,),
            in_specs=[pl.BlockSpec(memory_space=pl.ANY)] * 7,
            out_specs=pl.BlockSpec(memory_space=pl.ANY),
            out_shape=jax.ShapeDtypeStruct((S, D), BF),
            scratch_shapes=scratch,
            compiler_params=pltpu.CompilerParams(vmem_limit_bytes=120 * 2 ** 20),
            name="fused_block",
        )(A_x.reshape(S, D), A_wqkv, A_wo, B_w_r, B_w_gate, B_w_up, B_w_down)
        return out.reshape(1, S, D)

    return fused_block


_fused_block = build()


@jax.jit
def pallas_sequential_preLN__mha_block__moe_arch_mod__prompt_kernel(
    A_x: jax.Array,
    A_wqkv: jax.Array,
    A_wo: jax.Array,
    B_x: jax.Array,
    B_w_r: jax.Array,
    B_w_gate: jax.Array,
    B_w_up: jax.Array,
    B_w_down: jax.Array,
):
    return _fused_block(A_x, A_wqkv, A_wo, B_x, B_w_r, B_w_gate, B_w_up, B_w_down)
```

```python
import jax
import jax.numpy as jnp
import numpy as np
from jax import lax
import jax.experimental.pallas as pl
import jax.experimental.pallas.tpu as pltpu

S = 2048
D = 512
H = 32
DH = 16
F = 1792
EPS = 1e-5
QSCALE = DH ** -0.5 * 1.4426950408889634
HEADROOM = 40.0
L_MIN = 2.0 ** -64

W = 512
CH = 128
NB = CH // 8
NC = S // CH
NQ = S // W
TC = 512
TM = 128
TO = 128
OUT_CUTS = (0, 1152, 1792, 2048)

BF = jnp.bfloat16
F32 = jnp.float32
U32 = jnp.uint32
I32 = jnp.int32

VPU_PAIRS = (
    (4, 15), (8, 35), (25, 36), (39, 45), (51, 61), (58, 68), (71, 78), (83, 92),
    (85, 97), (104, 108), (115, 118), (126, 137), (133, 147), (141, 157), (153, 162), (169, 170),
    (178, 188), (187, 194), (202, 205), (213, 217), (221, 227), (231, 236), (245, 251))


def _pk(x):
    return pltpu.bitcast(x, U32)


def _upk(x):
    return pltpu.bitcast(x, BF)


def _dot(a, b, ca=1, cb=0):
    return lax.dot_general(a, b, (((ca,), (cb,)), ((), ())), preferred_element_type=F32)


def _center(x):
    xc = x - jnp.sum(x, axis=-1, keepdims=True) * (1.0 / D)
    return xc, lax.rsqrt(jnp.sum(xc * xc, axis=-1, keepdims=True) * (1.0 / D) + EPS)


def build(vpu_pairs=VPU_PAIRS, l_min=L_MIN):
    order = [NB * c + NB - 1 - j for c in range(NC) for j in range(NB)]
    vpu_blocks = [order[p] for pair in vpu_pairs for p in pair]
    mxu_blocks = [b for b in order if b not in vpu_blocks]
    mo = [1 + (sum(b // NB < c for b in mxu_blocks) + 1) // 2 for c in range(NC + 1)]
    vo = [sum(b // NB < c for b in vpu_blocks[::2]) for c in range(NC + 1)]
    mxu_blocks = vpu_blocks[:2] + mxu_blocks
    npair = len(vpu_pairs)

    def karray(n, a):
        return a * npair + n

    key_ops = [(d, i) for d in range(DH) for i in range((4 if d < 8 else 3) * npair)]
    key_cut = [len(key_ops) * i // (NQ * NC) for i in range(NQ * NC + 1)]

    def kslot(i, d):
        return i * DH + d + 1

    def qslot(u, i, t):
        return 4 * npair * DH + 4 + (2 * u + t) * 58 + i

    def kernel(x_hbm, wqkv_hbm, wo_hbm, wr_hbm, wg_hbm, wu_hbm, wd_hbm, out_hbm,
               x_v, wqkv_v, wo_v, wg_v, wu_v, wd_v, out_v,
               wt_s, qt_s, vt_s, xn_s, kv_s, kmax_s, ot_s, ka_s, op_s, qa_s, qs_s, nu_s, xf_s, hn_s,
               p_s, o_s, inv_s, zero_s, bad_s, wr_v, izero_s, sem, osem):
        def x_rows(i, r0, r1):
            rows = pl.ds(r0, r1 - r0)
            return pltpu.make_async_copy(x_hbm.at[rows], x_v.at[rows], sem.at[i])

        x_cp = [x_rows(0, 0, TC), x_rows(1, TC, 2 * TC), x_rows(2, 2 * TC, S)]
        w_cp = [pltpu.make_async_copy(wqkv_hbm.at[:, pl.ds(i * D, D)], wqkv_v.at[i], sem.at[3 + i])
                for i in range(3)]
        late = [pltpu.make_async_copy(src, dst, sem.at[6 + i]) for i, (src, dst) in enumerate(
            [(wo_hbm, wo_v), (wr_hbm, wr_v), (wg_hbm, wg_v), (wu_hbm, wu_v), (wd_hbm, wd_v)])]
        for cp in [x_cp[0], w_cp[1], w_cp[0], x_cp[1], w_cp[2], x_cp[2]] + late:
            cp.start()
        zero_s[...] = jnp.zeros_like(zero_s)
        p_s[...] = jnp.zeros_like(p_s)
        o_s[...] = jnp.zeros_like(o_s)
        inv_s[...] = jnp.ones_like(inv_s)
        bad_s[...] = jnp.zeros_like(bad_s)
        for i in range(izero_s.shape[0]):
            izero_s[i] = pl.program_id(0)

        def normalize(i):
            x = x_v[i * TC:(i + 1) * TC, :].astype(F32)
            xf_s[i * TC:(i + 1) * TC, :] = x
            xc, rstd = _center(x)
            xn = (xc * rstd).astype(BF)
            xn_s[i * TC // 2:(i + 1) * TC // 2, :] = _pk(xn)
            return xn

        kblk = {}

        def project_keys(i, xn):
            k = _dot(xn, wqkv_v[1])
            kblk.update({i * TC // 8 + b: k[8 * b:8 * b + 8] for b in range(TC // 8)})

        def largest(i, kmax):
            for b in range(i * TC // 8, (i + 1) * TC // 8):
                kmax = jnp.maximum(kmax, jnp.abs(kblk[b]))
            return kmax

        def arrange_keys(i):
            lane = lax.broadcasted_iota(I32, (8, 128), 1)
            for n in range(mo[NC]):
                pair = mxu_blocks[2 * n:2 * n + 2]
                if max(pair) // (TC // 8) != i:
                    continue
                km = _pk(jnp.concatenate([kblk[b] for b in pair], axis=0).astype(BF))
                for g in range(D // 128):
                    kg = km[:, g * 128:(g + 1) * 128]
                    for j in range(4):
                        kr = kg if j == 0 else pltpu.roll(kg, 128 - 2 * DH * j, 1)
                        for e in range(2):
                            ka_s[8 * g + 2 * j + e, 8 * n:8 * n + 8, :] = jnp.where(
                                lane == DH * (1 - e), np.uint32(0x3F803F80), kr)

        def arrange_vpu_keys(g, kmax):
            lo = lax.broadcasted_iota(I32, (8, 128), 1) % DH < 8
            inv = 1.0 / kmax
            for n in range(npair):
                k1, k2 = (kblk[b][:, g * 128:(g + 1) * 128] * inv for b in vpu_blocks[2 * n:2 * n + 2])
                s1 = k2 + pltpu.roll(k2, 120, 1)
                s2 = s1 - k1
                s3 = pltpu.roll(k1 - k2, 8, 1)
                s4 = pltpu.roll(k1, 120, 1) - s2
                for a, v in enumerate((k1, jnp.where(lo, s1, k2), jnp.where(lo, s2, s3), s4)):
                    kv_s[g, karray(n, a)] = v

        def project_t(i, part, jobs=()):
            cols = slice(i * TC, (i + 1) * TC)
            marks = []
            for r in range(0, D, TM):
                y = None
                for k in range(0, D, 128):
                    t = _dot(_upk(wt_s[part, r // 2:(r + TM) // 2, k:k + 128]),
                             _upk(xn_s[i * TC // 2:(i + 1) * TC // 2, k:k + 128]), 1, 1)
                    y = t if y is None else y + t
                    marks += [y[j:j + 8, :128] for j in range(0, TM, 8)]
                if part == 0:
                    qt_s[r:r + TM, cols] = y * QSCALE
                else:
                    vt_s[r // 2:(r + TM) // 2, cols] = _pk(y.astype(BF))
            for j, job in enumerate(jobs):
                spare = pl.ds(pl.multiple_of(izero_s[0] + D, 8), 8)
                kmax_s[spare, :] = marks[j * len(marks) // len(jobs)]
                bound(*job)

        def spread_keys(h, slot, dst):
            ops = key_ops[key_cut[slot]:key_cut[slot + 1]]
            for d in sorted({d for d, _ in ops}):
                arrays = [i for e, i in ops if e == d]
                k = kv_s[h >> 3, arrays[0]:arrays[-1] + 1].reshape(8 * len(arrays), 128)
                idx = jnp.full(k.shape, DH * (h & 7) + d, I32)
                k = jnp.take_along_axis(k, idx, axis=1, mode="promise_in_bounds")
                for j, i in enumerate(arrays):
                    dst[0, kslot(i, d)] = k[8 * j:8 * j + 8]

        def put_query(dst, u, i, v):
            for t in range(2):
                dst[0, qslot(u, i, t)] = v[:, t * 128:(t + 1) * 128]

        def query_terms(q):
            b11, b12, b21, b22 = q[:8, :W // 2], q[:8, W // 2:], q[8:, :W // 2], q[8:, W // 2:]
            t1 = b12 - b11
            t2 = b22 - t1
            return [b11, b21, t2, b22 - b12, b21 - t2, t1, b22]

        def spread_queries(terms, u, c, dst):
            for i in range(4 * c, min(4 * c + 4, 56)):
                put_query(dst, u, i, jnp.broadcast_to(terms[i // 8][i % 8:i % 8 + 1], (8, W // 2)))

        def bound(u, h):
            cols = slice(u * W, (u + 1) * W)
            q = qt_s[h * DH:(h + 1) * DH, cols]
            qs = q * jnp.concatenate([kmax_s[h * DH:(h + 1) * DH, :]] * (W // 128), axis=1)
            qs_s[h, u] = qs
            top = jnp.sum(jnp.abs(qs), axis=0, keepdims=True)
            top = jnp.broadcast_to(jnp.maximum(top[:, :W // 2], top[:, W // 2:]), (8, W // 2))
            bits = pltpu.bitcast(HEADROOM - top, U32) >> 16
            nu = pltpu.bitcast(bits << 16, F32)
            nu_s[h, u] = nu
            row = jnp.where(lax.broadcasted_iota(I32, (8, W // 2), 0) == 0, bits, np.uint32(0))
            qa_s[h, 8 * (h % 2):8 * (h % 2) + 8, cols] = _pk(q.astype(BF))
            qa_s[h, 8 - 8 * (h % 2):16 - 8 * (h % 2), cols] = jnp.concatenate([row, row], axis=1)
            if h == 0:
                put_query(op_s[0], u, 56, nu)
                for c in range(NC):
                    spread_queries(query_terms(qs), u, c, op_s[0])

        x_cp[0].wait()
        xn = normalize(0)
        w_cp[1].wait()
        project_keys(0, xn)
        w_cp[0].wait()
        x_cp[1].wait()
        wt_s[0] = _pk(wqkv_v[0].T)
        project_t(0, 0)
        kmax = largest(0, jnp.zeros((8, D), F32))
        arrange_keys(0)
        project_keys(1, normalize(1))
        w_cp[2].wait()
        x_cp[2].wait()
        project_t(1, 0)
        xn = normalize(2)
        wt_s[1] = _pk(wqkv_v[2].T)
        kmax = largest(1, kmax)
        arrange_keys(1)
        project_keys(2, xn)
        kmax = largest(2, kmax)
        project_t(0, 1)
        xn = normalize(3)
        arrange_keys(2)
        project_keys(3, xn)
        kmax = largest(3, kmax)
        kmax = jnp.maximum(jnp.max(kmax, axis=0, keepdims=True) * (1.0 + 2.0 ** -5), 2.0 ** -100)
        for g in range(D // 128):
            kmax_s[g * 128:(g + 1) * 128, :] = jnp.broadcast_to(kmax[:, g * 128:(g + 1) * 128], (128, 128)).T
        arrange_vpu_keys(0, kmax[:, :128])
        project_t(1, 1)
        arrange_keys(3)
        jobs = [(u, h) for u in range(NQ) for h in range(H)]
        job_cut = (0, 12, 50, 89, 128)
        for i, (chunk, part) in enumerate(((2, 0), (3, 0), (2, 1), (3, 1))):
            for slot in range(i * NC, (i + 1) * NC):
                spread_keys(0, slot, op_s[0])
            if i:
                arrange_vpu_keys(i, kmax[:, i * 128:(i + 1) * 128])
            project_t(chunk, part, jobs[job_cut[i]:job_cut[i + 1]])
        for cp in late:
            cp.wait()

        def weigh_values(h, u, c, p, o, inv):
            vc = vt_s[pl.ds(pl.multiple_of(jnp.maximum(h, 0) * 8, 8), 8), c * CH:(c + 1) * CH]
            o = o + _dot(_upk(vc), p)
            if c == NC - 1:
                out = o * jnp.concatenate([inv, inv], axis=0)
                ot_s[pl.ds(pl.multiple_of(h * 8 + 8, 8), 8), u * W:(u + 1) * W] = _pk(out.astype(BF))
            return o

        def head(h, src, dst):
            score, first_p = {}, {}
            z0 = pltpu.bitcast(zero_s[0:8, 0:128], I32)[0, 0]

            def mxu_scores(u, m0, m1):
                s = _dot(_upk(ka_s[h, 8 * m0:8 * m1, 0:2 * DH]), _upk(qa_s[h, :, u * W:(u + 1) * W]))
                for j, b in enumerate(mxu_blocks[2 * m0:2 * m1]):
                    score[u, b] = s[8 * j:8 * j + 8]

            def vpu_scores(u, j, z):
                def query(i):
                    return jnp.concatenate([src[z, qslot(u, i, t)] for t in range(2)], axis=1)

                def term(m, a, d0):
                    k = src[z, pl.ds(kslot(karray(j, a), d0), 8)]
                    return jnp.concatenate(
                        [jnp.sum(k * src[z, pl.ds(qslot(u, 8 * m, t), 8)], axis=0) for t in range(2)], axis=1)

                m1 = term(0, 0, 0) + query(56)
                c11 = term(1, 0, 8) + m1
                u2 = term(2, 2, 0) + m1
                m5 = term(5, 1, 0)
                c12 = term(6, 3, 0) + (u2 + m5)
                u3 = term(3, 2, 8) + u2
                c21 = term(4, 1, 8) + u3
                score[u, vpu_blocks[2 * j]] = jnp.concatenate([c11, c12], axis=1)
                score[u, vpu_blocks[2 * j + 1]] = jnp.concatenate([c21, u3 + m5], axis=1)

            def probabilities(u, c, l, terms):
                n = u * NC + c
                z = izero_s[n] + z0
                mxu_scores(u, mo[c] + 1 if n else 0, min(mo[c + 1] + 1, mo[NC]))
                if c == NC - 1 and u + 1 < NQ:
                    mxu_scores(u + 1, mo[0], mo[0] + 1)
                hn = jnp.minimum(h + 1, H - 1)
                if n >= 2:
                    dst[z, qslot(NQ, 0, 0)] = first_p[n - 2]
                if c == 0:
                    terms = query_terms(qs_s[hn, u])
                    put_query(dst, u, 56, nu_s[hn, u])
                spread_keys(hn, n, dst)
                spread_queries(terms, u, c, dst)
                for j in range(max(vo[c], 1 if u == 0 else 0), vo[c + 1]):
                    vpu_scores(u, j, z + izero_s[NQ * NC + j - vo[c] - 1] if j > vo[c] else z)
                p = {b: jnp.exp2(score.pop((u, NB * c + b))) for b in range(NB - 1, -1, -1)}
                first_p[n] = p[NB - 1][:, :128]
                for b in range(NB - 1, -1, -1):
                    l = p[b] if l is None else l + p[b]
                return jnp.concatenate([p[b] for b in range(NB)], axis=0), l, terms

            pending, o, l, bad = (h - 1, NQ - 1, NC - 1, p_s[...]), o_s[...], inv_s[...], bad_s[...]
            terms = None
            for u in range(NQ):
                for c in range(NC):
                    p, l_new, terms = probabilities(u, c, l if c else None, terms)
                    o = weigh_values(*pending, o, l)
                    if c == 0:
                        o = zero_s[...]
                    if c == NC - 1:
                        tot = jnp.broadcast_to(jnp.sum(l_new, axis=0, keepdims=True), (8, W))
                        for t in range(0, W, 128):
                            bad = jnp.where(tot[:, t:t + 128] >= l_min, bad, 1.0)
                        l_new = pltpu.reciprocal(tot, approx=True)
                        l_new = l_new * (2.0 - tot * l_new)
                    pending, l = (h, u, c, p), l_new
            p_s[...] = p
            o_s[...] = o
            inv_s[...] = l
            bad_s[...] = bad

        def two_heads(i, carry):
            head(2 * i, op_s[0], op_s[1])
            pl.when(izero_s[0] == 0)(lambda: head(2 * i + 1, op_s[1], op_s[0]))
            return carry

        lax.fori_loop(0, H // 2, two_heads, 0)

        @pl.when(jnp.max(bad_s[...]) > 0.0)
        def _with_true_maximum():
            def tile(t, carry):
                h = t // (S // 128)
                c0 = pl.multiple_of((h // 8) * 128, 128)
                q0 = pl.multiple_of((t % (S // 128)) * 128, 128)

                @pl.when(t % (8 * S // 128) == 0)
                def _():
                    @pl.loop(0, S // 128)
                    def _(r):
                        xn = _upk(xn_s[pl.ds(pl.multiple_of(r * 64, 64), 64), :])
                        rows = pl.ds(pl.multiple_of(r * 128, 128), 128)
                        hn_s[rows, 0:128] = _dot(xn, wqkv_v[1, :, pl.ds(c0, 128)])

                rows = lax.broadcasted_iota(I32, (128, 128), 0) // DH
                lanes = lax.broadcasted_iota(I32, (S, 128), 1) // DH
                qh = jnp.where(rows == h % 8, qt_s[pl.ds(c0, 128), pl.ds(q0, 128)], 0.0)
                kh = jnp.where(lanes == h % 8, hn_s[:, 0:128], 0.0)
                s = _dot(kh.astype(BF), qh.astype(BF))
                p = jnp.exp2(s - jnp.max(s, axis=0, keepdims=True))
                r8 = pl.multiple_of(h * 8, 8)
                o = _dot(_upk(vt_s[pl.ds(r8, 8), :]), p.astype(BF))
                o = o * (1.0 / jnp.sum(p, axis=0, keepdims=True))
                ot_s[pl.ds(r8 + 8, 8), pl.ds(q0, 128)] = _pk(o.astype(BF))
                o_s[:, pl.ds(pl.multiple_of(q0 % W, 128), 128)] = o
                return carry

            lax.fori_loop(0, H * (S // 128), tile, 0)
            p_s[...] = jnp.zeros_like(p_s)
            inv_s[...] = jnp.ones_like(inv_s)

        def out_cp(i):
            rows = pl.ds(OUT_CUTS[i], OUT_CUTS[i + 1] - OUT_CUTS[i])
            return pltpu.make_async_copy(out_v.at[rows], out_hbm.at[rows], osem.at[i])

        def attended(i):
            return _dot(_upk(ot_s[8:, i * TO:(i + 1) * TO]), wo_v[...], 0, 0)

        wr = wr_v[...].reshape(1, D).astype(F32)
        m1 = m2 = jnp.full((8, 1), -jnp.inf, F32)
        i1 = i2 = jnp.full((8, 1), -1, I32)
        att_next = attended(0)
        weigh_values(H - 1, NQ - 1, NC - 1, p_s[...], o_s[...], inv_s[...])
        for i in range(S // TO):
            rows = slice(i * TO, (i + 1) * TO)
            att = att_next
            if i + 1 < S // TO:
                att_next = attended(i + 1)
            h1 = xf_s[rows, :] + att
            hc, rstd = _center(h1)
            hn = hc * rstd
            hn_s[rows, :] = hn
            out_v[rows, :] = (h1 + hn).astype(BF)
            r = jnp.sum(hc * wr, axis=-1, keepdims=True) * rstd
            for j in range(TO // 8):
                n = i * TO // 8 + j
                rj = r[8 * j:8 * j + 8]
                gt1, gt2 = rj > m1, rj > m2
                m2, i2 = jnp.where(gt1, m1, jnp.where(gt2, rj, m2)), jnp.where(gt1, i1, jnp.where(gt2, n, i2))
                m1, i1 = jnp.where(gt1, rj, m1), jnp.where(gt1, n, i1)
            if (i + 1) * TO in OUT_CUTS:
                out_cp(OUT_CUTS.index((i + 1) * TO) - 1).start()

        sub = lax.broadcasted_iota(I32, (8, 1), 0)
        i1, i2 = (8 * i1 + sub).astype(F32), (8 * i2 + sub).astype(F32)

        def top(r, tok):
            m = jnp.max(r, axis=0, keepdims=True)
            return m, jnp.min(jnp.where(r == m, tok, S - 1.0), axis=0, keepdims=True)

        ra, fa = top(m1, i1)
        rb, fb = top(jnp.where(i1 == fa, m2, m1), jnp.where(i1 == fa, i2, i1))
        ta = jnp.clip(fa.astype(I32)[0, 0], 0, S - 1)
        tb = jnp.clip(fb.astype(I32)[0, 0], 0, S - 1)

        row16 = lax.broadcasted_iota(I32, (16, D), 0)
        xs = jnp.where(row16 == 0, hn_s[pl.ds(ta, 1), :], jnp.where(row16 == 1, hn_s[pl.ds(tb, 1), :], 0.0))
        xs = xs.astype(BF)
        gate = _dot(xs, wg_v[...])
        act = (gate * jax.nn.sigmoid(gate) * _dot(xs, wu_v[...])).astype(BF)
        y = _dot(act, wd_v[...])

        def tile_of(t):
            return pl.ds(pl.multiple_of((t // 16) * 16, 16), 16)

        for i in range(len(OUT_CUTS) - 1):
            out_cp(i).wait()
        for t, yr in ((ta, y[0:1] * jax.nn.sigmoid(ra)), (tb, y[1:2] * jax.nn.sigmoid(rb))):
            cur = out_v[tile_of(t), :].astype(F32)
            out_v[tile_of(t), :] = jnp.where(row16 == t % 16, cur + yr, cur).astype(BF)

        def fix_cp(t, i):
            return pltpu.make_async_copy(out_v.at[tile_of(t)], out_hbm.at[tile_of(t)], osem.at[i])

        fix_cp(ta, 0).start()

        @pl.when(ta // 16 != tb // 16)
        def _():
            fix_cp(tb, 1).start()
            fix_cp(tb, 1).wait()

        fix_cp(ta, 0).wait()

    scratch = [
        pltpu.VMEM((S, D), BF), pltpu.VMEM((3, D, D), BF), pltpu.VMEM((D, D), BF),
        pltpu.VMEM((D, F), BF), pltpu.VMEM((D, F), BF), pltpu.VMEM((F, D), BF), pltpu.VMEM((S, D), BF),
        pltpu.VMEM((2, D // 2, D), U32),
        pltpu.VMEM((D, S), F32),
        pltpu.VMEM((D // 2, S), U32),
        pltpu.VMEM((S // 2, D), U32),
        pltpu.VMEM((D // 128, 4 * npair, 8, 128), F32),
        pltpu.VMEM((D + 32, 128), F32),
        pltpu.VMEM((D // 2 + 8, S), U32),
        pltpu.VMEM((H, 32 * pl.cdiv(mo[NC], 4), 128), U32),
        [pltpu.VMEM((1, qslot(NQ, 4, 0), 8, 128), F32) for _ in range(2)],
        pltpu.VMEM((H, DH, S), U32),
        pltpu.VMEM((H, NQ, DH, W), F32),
        pltpu.VMEM((H, NQ, 8, W // 2), F32),
        pltpu.VMEM((S, D), F32), pltpu.VMEM((S, D), F32),
        pltpu.VMEM((CH, W), F32), pltpu.VMEM((DH, W), F32), pltpu.VMEM((8, W), F32),
        pltpu.VMEM((DH, W), F32), pltpu.VMEM((8, 128), F32), pltpu.VMEM((D,), BF),
        pltpu.SMEM((NQ * NC + 8,), I32),
        pltpu.SemaphoreType.DMA((11,)), pltpu.SemaphoreType.DMA((len(OUT_CUTS) - 1,)),
    ]

    def fused_block(A_x, A_wqkv, A_wo, B_x, B_w_r, B_w_gate, B_w_up, B_w_down):
        del B_x
        out = pl.pallas_call(
            kernel,
            grid=(1,),
            in_specs=[pl.BlockSpec(memory_space=pl.ANY)] * 7,
            out_specs=pl.BlockSpec(memory_space=pl.ANY),
            out_shape=jax.ShapeDtypeStruct((S, D), BF),
            scratch_shapes=scratch,
            compiler_params=pltpu.CompilerParams(vmem_limit_bytes=120 * 2 ** 20),
            name="fused_block",
        )(A_x.reshape(S, D), A_wqkv, A_wo, B_w_r, B_w_gate, B_w_up, B_w_down)
        return out.reshape(1, S, D)

    return fused_block


_fused_block = build()


@jax.jit
def pallas_sequential_preLN__mha_block__moe_arch_mod__prompt_kernel(
    A_x: jax.Array,
    A_wqkv: jax.Array,
    A_wo: jax.Array,
    B_x: jax.Array,
    B_w_r: jax.Array,
    B_w_gate: jax.Array,
    B_w_up: jax.Array,
    B_w_down: jax.Array,
):
    return _fused_block(A_x, A_wqkv, A_wo, B_x, B_w_r, B_w_gate, B_w_up, B_w_down)
```
